```python
import os as _os
_os.environ.setdefault("JAX_PLATFORMS", "cpu")
import jax
import jax.numpy as jnp

def _softmax(x, axis=-1):
    return jax.nn.softmax(x, axis=axis)
def _gelu(x):
    return jax.nn.gelu(x, approximate=True)
def _silu(x):
    return jax.nn.silu(x)
def _sigmoid(x):
    return jax.nn.sigmoid(x)
def _layernorm(x, axis=-1, eps=1e-5):
    m = jnp.mean(x, axis=axis, keepdims=True)
    v = jnp.var(x, axis=axis, keepdims=True)
    return (x - m) / jnp.sqrt(v + eps)
def _scatter_add(tgt, idx, src, axis=0):
    return tgt.at[idx].add(src)
def _segment_sum(src, seg, n):
    return jax.ops.segment_sum(src, seg, n)
class _Rng:
    def __init__(self, key):
        self._k = key
    def _next(self):
        self._k, sub = jax.random.split(self._k)
        return sub
    def normal(self, shape):
        return jax.random.normal(self._next(), shape, dtype=jnp.bfloat16)
    def randint(self, lo, hi, shape):
        return jax.random.randint(self._next(), shape, lo, hi, dtype=jnp.int32)
    def uniform(self, shape, lo=0.0, hi=1.0):
        return jax.random.uniform(self._next(), shape, jnp.bfloat16, lo, hi)
    def permutation(self, n):
        return jax.random.permutation(self._next(), n)


kernel_name = 'gated_mix__sliding_block__dense_activation_silu__prompt'

def setup_inputs():
    _rng = _Rng(jax.random.key(int.from_bytes(__import__("os").urandom(4), "little")))
    _w = (lambda a: (lambda t: t.astype(jnp.bfloat16) if jnp.issubdtype(t.dtype, jnp.floating) else t)(jnp.asarray(a)))
    def _A_setup():
        B, S, D = 1, 2048, 640
        return {
            "x": _w((lambda *s: _rng.normal(s) * 0.05)(B, S, D)),
            "wqkv": _w((lambda *s: _rng.normal(s) * 0.4)(D, 3 * D)),
            "wo": _w((lambda *s: _rng.normal(s) * 0.05)(D, D)),
        }
    _A_in = _A_setup()

    def _B_setup():
        B, S, D, F = 1, 2048, 640, 1536
        return {
            "x": _w((lambda *s: _rng.normal(s) * 0.05)(B, S, D)),
            "w1": _w((lambda *s: _rng.normal(s) * 1.6)(D, F) * (D ** -0.5)),
            "w2": _w((lambda *s: _rng.normal(s) * 1.6)(F, D) * (F ** -0.5)),
        }
    _B_in = _B_setup()

    return {
        "A_x": _A_in["x"],
        "A_wqkv": _A_in["wqkv"],
        "A_wo": _A_in["wo"],
        "B_x": _B_in["x"],
        "B_w1": _B_in["w1"],
        "B_w2": _B_in["w2"],
        "gate_w": _w((lambda *s: _rng.normal(s) * 0.05)(640) * 16.0),
    }

def reference(A_x, A_wqkv, A_wo, B_x, B_w1, B_w2, gate_w):
    def _A_ref(x, wqkv, wo):
        B, S, D = x.shape
        H = 32; Dh = D // H; W = 256
        qkv = (lambda x, *d: x.transpose(*d))((x @ wqkv).reshape(B, S, 3, H, Dh), 2, 0, 3, 1, 4)
        q, k, v = qkv[0], qkv[1], qkv[2]
        scores = jnp.einsum("bhqd,bhkd->bhqk", q, k) * (Dh ** -0.5)
        idx = jnp.arange(S)
        mask = (idx[:, None] - idx[None, :] >= 0) & (idx[:, None] - idx[None, :] < W)
        scores = jnp.where(mask[None, None], scores, -1e9)
        p = _softmax(scores, axis=-1)
        o = jnp.einsum("bhqk,bhkd->bhqd", p, v)
        return (lambda x, *d: x.transpose(*d))(o, 0, 2, 1, 3).reshape(B, S, D) @ wo

    def _B_ref(x, w1, w2):
        h = jnp.einsum("bsd,df->bsf", x, w1)
        h = _silu(h)
        out = jnp.einsum("bsf,fd->bsd", h, w2)
        return out

    x = A_x
    g = _sigmoid((x * gate_w).sum(-1, keepdims=True))
    a = _A_ref(x, A_wqkv, A_wo)
    b = _B_ref(x, B_w1, B_w2)
    return g * a + (1 - g) * b
```

```python
import functools
import math

import jax
import jax.numpy as jnp
import jax.experimental.pallas as pl
import jax.experimental.pallas.tpu as pltpu

S = 2048
D = 640
H = 32
DH = 20
W = 256
F = 1536
T = 512
G = 64
NPAIR = H // 2
PW = 2 * DH
VR = 48
KW = W + G
NEG = -1e30
EC = 128
NB = 32

_NT = (((1,), (1,)), ((), ()))


def _pair_loc(p):
    lo = PW * p
    if lo // 128 == (lo + PW - 1) // 128:
        return False, lo // 128, lo % 128
    lo -= 64
    assert lo // 128 == (lo + PW - 1) // 128
    return True, lo // 128, lo % 128


def _kernel(x_ref, wqkv_hbm, wo_hbm, w1_hbm, w2_hbm, gw_ref, o_ref,
            k_scr, kr_scr, vt_scr, q_scr, qr_scr, ot_scr, s_scr, r_scr,
            wqkv_ref, wo_ref, w1_ref, w2_ref, sems):
    i = pl.program_id(0)

    cp_qkv = pltpu.make_async_copy(wqkv_hbm, wqkv_ref, sems.at[0])
    cp_w1 = pltpu.make_async_copy(w1_hbm, w1_ref, sems.at[1])
    cp_w2 = pltpu.make_async_copy(w2_hbm, w2_ref, sems.at[2])
    cp_wo = pltpu.make_async_copy(wo_hbm, wo_ref, sems.at[3])

    @pl.when(i == 0)
    def _():
        cp_qkv.start()
        cp_w1.start()
        cp_w2.start()
        cp_wo.start()
        cp_qkv.wait()

    f32 = jnp.float32
    bf16 = jnp.bfloat16
    u32 = jnp.uint32

    x = x_ref[...]
    row0 = pl.multiple_of(i * T, T)

    qscale = (DH ** -0.5) * math.log2(math.e)
    v = jnp.dot(x, wqkv_ref[:, 2 * D:3 * D], preferred_element_type=f32)
    vt = v.T
    tail = (jax.lax.broadcasted_iota(jnp.int32, (8, 128), 0) == 0).astype(f32)
    for b in range(T // 128):
        blk = i * (T // 128) + b + 2
        for p in range(NPAIR):
            piece = jnp.concatenate(
                [vt[PW * p:PW * (p + 1), 128 * b:128 * (b + 1)], tail], axis=0)
            vt_scr[blk, VR * p:VR * (p + 1), :] = piece.astype(bf16)

    k = jnp.dot(x, wqkv_ref[:, D:2 * D], preferred_element_type=f32)
    k_scr[pl.ds(row0 + W, T), :] = k.astype(bf16)
    kr_scr[pl.ds(row0 + W, T), :] = k[:, 64:576].astype(bf16)
    q = jnp.dot(x, wqkv_ref[:, 0:D], preferred_element_type=f32) * qscale
    q_scr[...] = q.astype(bf16)
    qr_scr[...] = q[:, 64:576].astype(bf16)

    @pl.when(i == 0)
    def _():
        k_scr[0:W, :] = jnp.broadcast_to(k_scr[W:W + 1, :], (W, D))
        kr_scr[0:W, :] = jnp.broadcast_to(kr_scr[W:W + 1, :], (W, 512))
        vt_scr[0:2] = jnp.zeros((2, NPAIR * VR, 128), bf16)
        cp_w1.wait()
        cp_w2.wait()
        cp_wo.wait()

    h = jnp.dot(x, w1_ref[...], preferred_element_type=f32)
    h = (h * jax.nn.sigmoid(h)).astype(bf16)

    r_idx = jax.lax.broadcasted_iota(jnp.int32, (G, 128), 0)
    jm = jax.lax.broadcasted_iota(jnp.int32, (G, 128), 1) % G
    lo_ok = r_idx > jm
    hi_ok = r_idx <= jm
    lane_p = jax.lax.broadcasted_iota(jnp.int32, (G // 2, 128), 1)
    row40 = jax.lax.broadcasted_iota(jnp.int32, (PW, 128), 0)
    lane40 = jax.lax.broadcasted_iota(jnp.int32, (PW, 128), 1)

    tiles = [(g, p) for g in range(T // G) for p in range(NPAIR)]
    nbatch = len(tiles) // NB

    def qk(t, slot):
        g, p = tiles[t]
        ql = G * g
        q0 = row0 + ql
        rot, c, off = _pair_loc(p)
        ksrc = kr_scr if rot else k_scr
        qsrc = qr_scr if rot else q_scr
        kwin = ksrc[pl.ds(pl.multiple_of(q0, G), KW), 128 * c:128 * (c + 1)]
        qg = pltpu.bitcast(qsrc[ql:ql + G, 128 * c:128 * (c + 1)], u32)
        zero = jnp.zeros_like(qg)
        qa = jnp.where((lane_p >= off) & (lane_p < off + DH), qg, zero)
        qb = jnp.where((lane_p >= off + DH) & (lane_p < off + PW), qg, zero)
        qm = pltpu.bitcast(jnp.concatenate([qa, qb], axis=0), bf16)
        s_scr[slot] = jax.lax.dot_general(kwin, qm, _NT, preferred_element_type=f32)

    def sm_pv(t, slot):
        g, p = tiles[t]
        blk, half = g // 2, g % 2
        s_lo = jnp.where(lo_ok, s_scr[slot, 0:G, :], NEG)
        s_hi = jnp.where(hi_ok, s_scr[slot, W:KW, :], NEG)
        if half == 0:
            sa = jnp.concatenate([s_lo, s_scr[slot, G:128, :]], axis=0)
            sb = s_scr[slot, 128:W, :]
            sc = s_hi
        else:
            sa = s_lo
            sb = s_scr[slot, G:192, :]
            sc = jnp.concatenate([s_scr[slot, 192:W, :], s_hi], axis=0)
        m = jnp.maximum(jnp.maximum(jnp.max(sa, axis=0, keepdims=True),
                                    jnp.max(sb, axis=0, keepdims=True)),
                        jnp.max(sc, axis=0, keepdims=True))
        pa = jnp.exp2(sa - m).astype(bf16)
        pb = jnp.exp2(sb - m).astype(bf16)
        pc = jnp.exp2(sc - m).astype(bf16)
        kb = i * (T // 128) + blk
        v0 = vt_scr[kb, VR * p:VR * (p + 1), :]
        v1 = vt_scr[kb + 1, VR * p:VR * (p + 1), :]
        v2 = vt_scr[kb + 2, VR * p:VR * (p + 1), :]
        if half == 0:
            v2 = v2[:, 0:64]
        else:
            v0 = v0[:, 64:128]
        acc = jnp.dot(v0, pa, preferred_element_type=f32)
        acc += jnp.dot(v1, pb, preferred_element_type=f32)
        acc += jnp.dot(v2, pc, preferred_element_type=f32)
        res = acc[0:PW] / acc[PW:PW + 1]
        if half == 0:
            r_scr[p] = res
        else:
            a, b = r_scr[p], res
            top = row40 < DH
            keep = jnp.where(top, a, b)
            move = jnp.where(top, b, a)
            move = pltpu.roll(move, 64, 1)
            ot_scr[PW * p:PW * (p + 1), 128 * blk:128 * (blk + 1)] = jnp.where(
                (lane40 < G) == top, keep, move)

    for j in range(NB):
        qk(j, j)
    for b in range(nbatch):
        if b + 1 < nbatch:
            for j in range(NB):
                qk((b + 1) * NB + j, ((b + 1) % 2) * NB + j)
        for j in range(NB):
            sm_pv(b * NB + j, (b % 2) * NB + j)

    y = jnp.dot(h, w2_ref[...], preferred_element_type=f32)
    gwf = gw_ref[...].astype(f32).reshape(1, D)
    for r in range(T // EC):
        rows = slice(EC * r, EC * (r + 1))
        o = ot_scr[:, rows].T.astype(bf16)
        att = jnp.dot(o, wo_ref[...], preferred_element_type=f32)
        gl = jnp.sum(x_ref[rows, :].astype(f32) * gwf, axis=-1, keepdims=True)
        g = jax.nn.sigmoid(gl)
        o_ref[rows, :] = (g * att + (1.0 - g) * y[rows]).astype(o_ref.dtype)


@jax.jit
def pallas_gated_mix__sliding_block__dense_activation_silu__prompt_kernel(
    A_x, A_wqkv, A_wo, B_x, B_w1, B_w2, gate_w):
    x = A_x.reshape(S, D)
    gw = gate_w
    bf16 = jnp.bfloat16
    full = lambda shape: pl.BlockSpec(shape, lambda i: (0,) * len(shape))
    out = pl.pallas_call(
        _kernel,
        grid=(S // T,),
        in_specs=[
            pl.BlockSpec((T, D), lambda i: (i, 0)),
            pl.BlockSpec(memory_space=pl.ANY),
            pl.BlockSpec(memory_space=pl.ANY),
            pl.BlockSpec(memory_space=pl.ANY),
            pl.BlockSpec(memory_space=pl.ANY),
            full((D,)),
        ],
        out_specs=pl.BlockSpec((T, D), lambda i: (i, 0)),
        out_shape=jax.ShapeDtypeStruct((S, D), bf16),
        scratch_shapes=[
            pltpu.VMEM((S + W, D), bf16),
            pltpu.VMEM((S + W, 512), bf16),
            pltpu.VMEM((S // 128 + 2, NPAIR * VR, 128), bf16),
            pltpu.VMEM((T, D), bf16),
            pltpu.VMEM((T, 512), bf16),
            pltpu.VMEM((D, T), jnp.float32),
            pltpu.VMEM((2 * NB, KW, 128), jnp.float32),
            pltpu.VMEM((NPAIR, PW, 128), jnp.float32),
            pltpu.VMEM((D, 3 * D), bf16),
            pltpu.VMEM((D, D), bf16),
            pltpu.VMEM((D, F), bf16),
            pltpu.VMEM((F, D), bf16),
            pltpu.SemaphoreType.DMA((4,)),
        ],
        compiler_params=pltpu.CompilerParams(
            dimension_semantics=("arbitrary",),
            vmem_limit_bytes=100 * 1024 * 1024,
        ),
    )(x, A_wqkv, A_wo, B_w1, B_w2, gw)
    return out.reshape(1, S, D)
```

```python
import math

import jax
import jax.numpy as jnp
import jax.experimental.pallas as pl
import jax.experimental.pallas.tpu as pltpu

S = 2048
D = 640
H = 32
DH = 20
W = 256
F = 1536
T = 512
G = 64
NPAIR = H // 2
PW = 2 * DH
VR = 48
KW = W + G
NEG = -1e30
EC = 128
NB = 16

_NT = (((1,), (1,)), ((), ()))


def _pair_loc(p):
    lo = PW * p
    if lo // 128 == (lo + PW - 1) // 128:
        return False, lo // 128, lo % 128
    lo -= 64
    assert lo // 128 == (lo + PW - 1) // 128
    return True, lo // 128, lo % 128


def _kernel(x_hbm, wqkv_hbm, wo_hbm, w1_hbm, w2_hbm, gw_ref, o_hbm,
            k_scr, kr_scr, vt_scr, q_scr, qr_scr, ot_scr, s_scr, r_scr,
            wqkv_ref, wo_ref, w1_ref, w2_ref, sems, x_buf, o_buf, osems):
    f32 = jnp.float32
    bf16 = jnp.bfloat16
    u32 = jnp.uint32

    i = pl.program_id(0)
    nsteps = pl.num_programs(0)
    slot = i % 2

    cp_qkv = pltpu.make_async_copy(wqkv_hbm, wqkv_ref, sems.at[0])
    cp_w1 = pltpu.make_async_copy(w1_hbm, w1_ref, sems.at[1])
    cp_w2 = pltpu.make_async_copy(w2_hbm, w2_ref, sems.at[2])
    cp_wo = pltpu.make_async_copy(wo_hbm, wo_ref, sems.at[3])

    def x_copy(step, sl):
        return pltpu.make_async_copy(
            x_hbm.at[pl.ds(pl.multiple_of(step * T, T), T)], x_buf.at[sl],
            sems.at[4 + sl])

    def o_copy(step, sl, r):
        return pltpu.make_async_copy(
            o_buf.at[sl, EC * r:EC * (r + 1)],
            o_hbm.at[pl.ds(pl.multiple_of(step * T + EC * r, EC), EC)],
            osems.at[sl, r])

    @pl.when(i == 0)
    def _():
        cp_qkv.start()
        x_copy(0, 0).start()
        cp_w1.start()
        cp_w2.start()
        cp_wo.start()
        cp_qkv.wait()

    x_copy(i, slot).wait()

    @pl.when(i + 1 < nsteps)
    def _():
        x_copy(i + 1, 1 - slot).start()

    @pl.when(i >= 2)
    def _():
        for r in range(T // EC):
            o_copy(i - 2, slot, r).wait()

    x_ref = x_buf.at[slot]
    x = x_ref[...]
    row0 = pl.multiple_of(i * T, T)

    qscale = (DH ** -0.5) * math.log2(math.e)
    v = jnp.dot(x, wqkv_ref[:, 2 * D:3 * D], preferred_element_type=f32)
    vt = v.T
    tail = (jax.lax.broadcasted_iota(jnp.int32, (8, 128), 0) == 0).astype(f32)
    for b in range(T // 128):
        blk = i * (T // 128) + b + 2
        for p in range(NPAIR):
            piece = jnp.concatenate(
                [vt[PW * p:PW * (p + 1), 128 * b:128 * (b + 1)], tail], axis=0)
            vt_scr[blk, VR * p:VR * (p + 1), :] = piece.astype(bf16)

    k = jnp.dot(x, wqkv_ref[:, D:2 * D], preferred_element_type=f32)
    k_scr[pl.ds(row0 + W, T), :] = k.astype(bf16)
    kr_scr[pl.ds(row0 + W, T), :] = k[:, 64:576].astype(bf16)
    q = jnp.dot(x, wqkv_ref[:, 0:D], preferred_element_type=f32) * qscale
    q_scr[...] = q.astype(bf16)
    qr_scr[...] = q[:, 64:576].astype(bf16)

    @pl.when(i == 0)
    def _():
        k_scr[0:W, :] = jnp.broadcast_to(k_scr[W:W + 1, :], (W, D))
        kr_scr[0:W, :] = jnp.broadcast_to(kr_scr[W:W + 1, :], (W, 512))
        vt_scr[0:2] = jnp.zeros((2, NPAIR * VR, 128), bf16)
        cp_w1.wait()
        cp_w2.wait()
        cp_wo.wait()

    h = jnp.dot(x, w1_ref[...], preferred_element_type=f32)
    h = (h * jax.nn.sigmoid(h)).astype(bf16)

    r_idx = jax.lax.broadcasted_iota(jnp.int32, (G, 128), 0)
    jm = jax.lax.broadcasted_iota(jnp.int32, (G, 128), 1) % G
    lo_ok = r_idx > jm
    hi_ok = r_idx <= jm
    lane_p = jax.lax.broadcasted_iota(jnp.int32, (G // 2, 128), 1)
    row40 = jax.lax.broadcasted_iota(jnp.int32, (PW, 128), 0)
    lane40 = jax.lax.broadcasted_iota(jnp.int32, (PW, 128), 1)

    tiles = [(g, p) for g in range(T // G) for p in range(NPAIR)]

    def qk(t, sslot):
        g, p = tiles[t]
        ql = G * g
        q0 = row0 + ql
        rot, c, off = _pair_loc(p)
        ksrc = kr_scr if rot else k_scr
        qsrc = qr_scr if rot else q_scr
        kwin = ksrc[pl.ds(pl.multiple_of(q0, G), KW), 128 * c:128 * (c + 1)]
        qg = pltpu.bitcast(qsrc[ql:ql + G, 128 * c:128 * (c + 1)], u32)
        zero = jnp.zeros_like(qg)
        qa = jnp.where((lane_p >= off) & (lane_p < off + DH), qg, zero)
        qb = jnp.where((lane_p >= off + DH) & (lane_p < off + PW), qg, zero)
        qm = pltpu.bitcast(jnp.concatenate([qa, qb], axis=0), bf16)
        s_scr[sslot] = jax.lax.dot_general(kwin, qm, _NT, preferred_element_type=f32)

    def sm_pv(t, sslot):
        g, p = tiles[t]
        blk, half = g // 2, g % 2
        s_lo = jnp.where(lo_ok, s_scr[sslot, 0:G, :], NEG)
        s_hi = jnp.where(hi_ok, s_scr[sslot, W:KW, :], NEG)
        if half == 0:
            sa = jnp.concatenate([s_lo, s_scr[sslot, G:128, :]], axis=0)
            sb = s_scr[sslot, 128:W, :]
            sc = s_hi
        else:
            sa = s_lo
            sb = s_scr[sslot, G:192, :]
            sc = jnp.concatenate([s_scr[sslot, 192:W, :], s_hi], axis=0)
        m = jnp.maximum(jnp.maximum(jnp.max(sa, axis=0, keepdims=True),
                                    jnp.max(sb, axis=0, keepdims=True)),
                        jnp.max(sc, axis=0, keepdims=True))
        pa = jnp.exp2(sa - m).astype(bf16)
        pb = jnp.exp2(sb - m).astype(bf16)
        pc = jnp.exp2(sc - m).astype(bf16)
        kb = i * (T // 128) + blk
        v0 = vt_scr[kb, VR * p:VR * (p + 1), :]
        v1 = vt_scr[kb + 1, VR * p:VR * (p + 1), :]
        v2 = vt_scr[kb + 2, VR * p:VR * (p + 1), :]
        if half == 0:
            v2 = v2[:, 0:64]
        else:
            v0 = v0[:, 64:128]
        acc = jnp.dot(v0, pa, preferred_element_type=f32)
        acc += jnp.dot(v1, pb, preferred_element_type=f32)
        acc += jnp.dot(v2, pc, preferred_element_type=f32)
        res = acc[0:PW] / acc[PW:PW + 1]
        if half == 0:
            r_scr[p] = res
        else:
            a, b = r_scr[p], res
            top = row40 < DH
            keep = jnp.where(top, a, b)
            move = jnp.where(top, b, a)
            move = pltpu.roll(move, 64, 1)
            ot_scr[PW * p:PW * (p + 1), 128 * blk:128 * (blk + 1)] = jnp.where(
                (lane40 < G) == top, keep, move)

    nt = len(tiles)
    for j in range(NB):
        qk(j, j % (2 * NB))
    for t in range(nt):
        if t + NB < nt:
            qk(t + NB, (t + NB) % (2 * NB))
        sm_pv(t, t % (2 * NB))

    y = jnp.dot(h, w2_ref[...], preferred_element_type=f32)
    gwf = gw_ref[...].astype(f32).reshape(1, D)
    for r in range(T // EC):
        rows = slice(EC * r, EC * (r + 1))
        o = ot_scr[:, rows].T.astype(bf16)
        att = jnp.dot(o, wo_ref[...], preferred_element_type=f32)
        gl = jnp.sum(x_ref[rows, :].astype(f32) * gwf, axis=-1, keepdims=True)
        g = jax.nn.sigmoid(gl)
        o_buf[slot, rows, :] = (g * att + (1.0 - g) * y[rows]).astype(bf16)
        o_copy(i, slot, r).start()

    @pl.when(i == nsteps - 1)
    def _():
        for r in range(T // EC):
            o_copy(i - 1, 1 - slot, r).wait()
            o_copy(i, slot, r).wait()


@jax.jit
def pallas_gated_mix__sliding_block__dense_activation_silu__prompt_kernel(
    A_x: jax.Array,
    A_wqkv: jax.Array,
    A_wo: jax.Array,
    B_x: jax.Array,
    B_w1: jax.Array,
    B_w2: jax.Array,
    gate_w: jax.Array,
):
    assert A_x.shape == (1, S, D) and A_wqkv.shape == (D, 3 * D)
    assert A_wo.shape == (D, D) and B_w1.shape == (D, F) and B_w2.shape == (F, D)
    bf16 = jnp.bfloat16
    x = A_x.reshape(S, D)
    out = pl.pallas_call(
        _kernel,
        grid=(S // T,),
        in_specs=[
            pl.BlockSpec(memory_space=pl.ANY),
            pl.BlockSpec(memory_space=pl.ANY),
            pl.BlockSpec(memory_space=pl.ANY),
            pl.BlockSpec(memory_space=pl.ANY),
            pl.BlockSpec(memory_space=pl.ANY),
            pl.BlockSpec((D,), lambda i: (0,)),
        ],
        out_specs=pl.BlockSpec(memory_space=pl.ANY),
        out_shape=jax.ShapeDtypeStruct((S, D), bf16),
        scratch_shapes=[
            pltpu.VMEM((S + W, D), bf16),
            pltpu.VMEM((S + W, 512), bf16),
            pltpu.VMEM((S // 128 + 2, NPAIR * VR, 128), bf16),
            pltpu.VMEM((T, D), bf16),
            pltpu.VMEM((T, 512), bf16),
            pltpu.VMEM((D, T), jnp.float32),
            pltpu.VMEM((2 * NB, KW, 128), jnp.float32),
            pltpu.VMEM((NPAIR, PW, 128), jnp.float32),
            pltpu.VMEM((D, 3 * D), bf16),
            pltpu.VMEM((D, D), bf16),
            pltpu.VMEM((D, F), bf16),
            pltpu.VMEM((F, D), bf16),
            pltpu.SemaphoreType.DMA((6,)),
            pltpu.VMEM((2, T, D), bf16),
            pltpu.VMEM((2, T, D), bf16),
            pltpu.SemaphoreType.DMA((2, T // EC)),
        ],
        compiler_params=pltpu.CompilerParams(
            dimension_semantics=("arbitrary",),
            vmem_limit_bytes=100 * 1024 * 1024,
        ),
    )(x, A_wqkv, A_wo, B_w1, B_w2, gate_w)
    return out.reshape(1, S, D)
```
